```python
import jax
import jax.numpy as jnp

def _softmax(x, axis=-1):
    return jax.nn.softmax(x, axis=axis)

def _gelu(x):
    return jax.nn.gelu(x, approximate=True)

def _silu(x):
    return jax.nn.silu(x)

def _sigmoid(x):
    return jax.nn.sigmoid(x)

def _layernorm(x, axis=-1, eps=1e-05):
    m = jnp.mean(x, axis=axis, keepdims=True)
    v = jnp.var(x, axis=axis, keepdims=True)
    return (x - m) / jnp.sqrt(v + eps)

def _scatter_add(tgt, idx, src, axis=0):
    return tgt.at[idx].add(src)

def _segment_sum(src, seg, n):
    return jax.ops.segment_sum(src, seg, n)

class _Rng:

    def __init__(self, key):
        self._k = key

    def _next(self):
        self._k, sub = jax.random.split(self._k)
        return sub

    def normal(self, shape):
        return jax.random.normal(self._next(), shape, dtype=jnp.bfloat16)

    def randint(self, lo, hi, shape):
        return jax.random.randint(self._next(), shape, lo, hi, dtype=jnp.int32)

    def uniform(self, shape, lo=0.0, hi=1.0):
        return jax.random.uniform(self._next(), shape, jnp.bfloat16, lo, hi)

    def permutation(self, n):
        return jax.random.permutation(self._next(), n)
kernel_name = 'standalone__window_attn_davit__vision'

def setup_inputs():
    _rng = _Rng(jax.random.key(int.from_bytes(__import__("os").urandom(4), "little")))
    _w = lambda a: (lambda t: t.astype(jnp.bfloat16) if jnp.issubdtype(t.dtype, jnp.floating) else t)(jnp.asarray(a))
    HW = 512
    C0 = 192
    ws = 7
    nh = 4
    H = W = max(HW // ws * ws, ws)
    C = max(C0 // nh * nh, nh)
    k = 3
    return {'x': _w((lambda *s: _rng.normal(s) * 0.05)(1, H, W, C)), 'dw_pe': _w((lambda *s: _rng.normal(s) * 0.05)(k, k, C) * 0.1), 'w_qkv': _w((lambda *s: _rng.normal(s) * 0.05)(C, 3 * C) * C ** (-0.5)), 'w_o': _w((lambda *s: _rng.normal(s) * 0.05)(C, C) * C ** (-0.5))}

def reference(x, dw_pe, w_qkv, w_o):
    B, H, W, C = x.shape
    ws = 7
    nh = 4
    dh = C // nh
    kk = dw_pe.shape[0]
    pad = kk // 2
    xp = jnp.pad(x, ((0, 0), (pad, pad), (pad, pad), (0, 0)))
    pe = jnp.zeros_like(x)
    for i in range(kk):
        for j in range(kk):
            pe = pe + xp[:, i:i + H, j:j + W, :] * dw_pe[i, j][None, None, None, :]
    x0 = x + pe
    h = _layernorm(x0, axis=-1)
    hw = h.reshape(B, H // ws, ws, W // ws, ws, C)
    hw = (lambda x, *d: x.transpose(*d))(hw, 0, 1, 3, 2, 4, 5)
    hw = hw.reshape(-1, ws * ws, C)
    qkv = (hw @ w_qkv).reshape(-1, ws * ws, 3, nh, dh)
    q = qkv[:, :, 0].copy()
    k = qkv[:, :, 1].copy()
    v = qkv[:, :, 2].copy()
    scale = dh ** (-0.5)
    attn = jnp.einsum('wnhd,wmhd->whnm', q, k) * scale
    attn = _softmax(attn, axis=-1)
    out = jnp.einsum('whnm,wmhd->wnhd', attn, v)
    out = out.reshape(-1, ws * ws, C) @ w_o
    out = out.reshape(B, H // ws, W // ws, ws, ws, C)
    out = (lambda x, *d: x.transpose(*d))(out, 0, 1, 3, 2, 4, 5)
    out = out.reshape(B, H, W, C)
    return x0 + out
```

```python
import functools
import os
import numpy as np
import jax
import jax.numpy as jnp
import jax.experimental.pallas as pl
import jax.experimental.pallas.tpu as pltpu

WS = 7
NH = 4
C = 192
DH = C // NH
H = W = 511
WP = 512
NW = W // WS
EPS = 1e-05
NEG = -1e30
F32 = jnp.float32
BF16 = jnp.bfloat16


def _nt(a, b):
    return jax.lax.dot_general(a, b, (((1,), (1,)), ((), ())), preferred_element_type=F32)


def _nn(a, b):
    return jax.lax.dot_general(a, b, (((1,), (0,)), ((), ())), preferred_element_type=F32)


def _kernel(xt_ref, xm_ref, xb_ref, dw_ref, wqkv_ref, wo_ref, o_ref,
            wq_s, wo_s, dwb_s, x0_e, x0_o, qkv_e, qkv_o, att_e, att_o):
    r = pl.program_id(0)

    @pl.when(r == 0)
    def _prep():
        w = wqkv_ref[...].astype(F32)
        qs = w[:, 0:C] * np.float32(DH ** -0.5 * np.log2(np.e))
        q = [qs[:, h * DH:(h + 1) * DH] for h in range(NH)]
        k = [w[:, C + h * DH:C + (h + 1) * DH] for h in range(NH)]
        v = [w[:, 2 * C + h * DH:2 * C + (h + 1) * DH] for h in range(NH)]
        z32 = jnp.zeros((C, 32), F32)
        tiles = [
            [q[0], v[2][:, 32:48], v[3][:, 0:16], q[1]],
            [v[2][:, 0:32], q[2], q[3]],
            [k[0], z32, k[1]],
            [z32, k[2], k[3]],
            [v[0], v[1], v[3][:, 16:48]],
        ]
        for t in range(5):
            wq_s[:, t * 128:(t + 1) * 128] = jnp.concatenate(tiles[t], axis=1).astype(BF16)
        wo = wo_ref[...].astype(F32)
        zr = lambda n: jnp.zeros((n, C), F32)
        wo2 = jnp.concatenate([
            wo[0:96], zr(32),
            wo[96:128], zr(16), wo[128:144], wo[144:160], zr(16), wo[160:192]], axis=0)
        wo_s[...] = wo2.T.astype(BF16)
        dw = dw_ref[...].astype(F32)
        for j in range(9):
            col = dw[:, j:j + 1]
            if j == 4:
                col = col + 1.0
            dwb_s[j] = jnp.broadcast_to(col, (C, 128))

        x0_e[...] = jnp.zeros(x0_e.shape, F32)
        x0_o[...] = jnp.zeros(x0_o.shape, F32)
        qkv_e[...] = jnp.zeros(qkv_e.shape, F32)
        att_o[...] = jnp.ones(att_o.shape, F32)

    NI = int(os.environ.get('NI', '4'))
    NT = 4 // NI
    NG = 12 // NI
    NWI = -(-NW // NI)
    lane16 = jax.lax.broadcasted_iota(jnp.int32, (16, 128), 1)
    l8 = jax.lax.broadcasted_iota(jnp.int32, (8, 128), 1)
    seg_a = l8 < 64
    key_ok = jnp.logical_and((l8 % 64) < 56, (l8 % 8) < 7)
    oka = jnp.logical_and(key_ok, seg_a)
    okb = jnp.logical_and(key_ok, jnp.logical_not(seg_a))
    ra = jnp.minimum(r, NW - 1)
    top_ok = ra > 0
    bot_ok = ra < NW - 1

    def between(lo, hi):
        return jnp.logical_and(l8 >= lo, l8 < hi)

    def ones_at(lo, hi):
        return jnp.where(between(lo, hi), 1.0, 0.0).astype(F32)

    def slot(q):
        return ((q + 4) // 2) % 2

    def stage_a(x0_s, g):
        cs = pl.ds(pl.multiple_of(g * 16, 16), 16)
        base = slot(r) * (WS * 4)
        wts = [dwb_s[j, cs, :] for j in range(9)]

        def load_row(i):
            if i == -1:
                v = jnp.where(top_ok, xt_ref[0, cs, :].astype(F32), 0.0)
            elif i == WS:
                v = jnp.where(bot_ok, xb_ref[0, cs, :].astype(F32), 0.0)
            else:
                v = xm_ref[i, cs, :].astype(F32)
            parts = [v[:, t * 128:(t + 1) * 128] for t in range(4)]
            parts[3] = jnp.where(lane16 < 127, parts[3], 0.0)
            return parts

        rows = {-1: load_row(-1), 0: load_row(0)}
        for i in range(WS):
            rows[i + 1] = load_row(i + 1)
            v0, v1, v2 = [], [], []
            for t in range(4):
                a, b, c = rows[i - 1][t], rows[i][t], rows[i + 1][t]
                v0.append(pltpu.roll(a * wts[0] + b * wts[3] + c * wts[6], 1, 1))
                v1.append(a * wts[1] + b * wts[4] + c * wts[7])
                v2.append(pltpu.roll(a * wts[2] + b * wts[5] + c * wts[8], 127, 1))
            for t in range(4):
                l = jnp.where(lane16 == 0, 0.0 if t == 0 else v0[t - 1], v0[t])
                rr = jnp.where(lane16 == 127, 0.0 if t == 3 else v2[t + 1], v2[t])
                x0_s[base + (i * 4 + t), cs, :] = v1[t] + l + rr
            del rows[i - 1]

    def stage_l(x0_s, qkv_s, i, t):
        x0 = x0_s[slot(r - 1) * (WS * 4) + i * 4 + t]
        m = jnp.mean(x0, axis=0, keepdims=True)
        d = x0 - m
        var = jnp.mean(d * d, axis=0, keepdims=True)
        h = d * jax.lax.rsqrt(var + EPS)
        ht = h.T.astype(BF16)
        qkv = _nn(ht, wq_s[...])
        rows = pl.ds(pl.multiple_of(i * WP + t * 128, 128), 128)
        for j in range(5):
            qkv_s[j, rows, :] = qkv[:, j * 128:(j + 1) * 128]

    z8 = jnp.zeros((8, 128), F32)

    def ext(rows_a, rows_b):
        return jnp.concatenate(rows_a + [z8] + rows_b + [z8], axis=0).astype(BF16)

    def stage_b(qkv_s, att_s, c):
        def ld(t):
            return [qkv_s[t, pl.ds(i * WP + c * WS, 8), :] for i in range(WS)]

        t0, t1, t2, t3, t4 = ld(0), ld(1), ld(2), ld(3), ld(4)
        q01 = jnp.concatenate(t0, axis=0).astype(BF16)
        q23 = jnp.concatenate(t1, axis=0).astype(BF16)
        k01 = ext([jnp.where(l8 < 48, x, 0.0) for x in t2], [jnp.where(l8 >= 80, x, 0.0) for x in t2])
        k23 = ext([jnp.where(between(32, 80), x, 0.0) for x in t3], [jnp.where(l8 >= 80, x, 0.0) for x in t3])
        v01 = ext([jnp.where(l8 < 48, x, ones_at(96, 112)) for x in t4],
                  [jnp.where(between(48, 96), x, ones_at(112, 128)) for x in t4])
        v23 = ext([jnp.where(l8 < 32, b, jnp.where(between(48, 64), a, ones_at(32, 48))) for a, b in zip(t0, t1)],
                  [jnp.where(l8 >= 96, d, jnp.where(between(64, 80), a, ones_at(80, 96))) for a, d in zip(t0, t4)])
        for t, (q, k, v) in enumerate(((q01, k01, v01), (q23, k23, v23))):
            s = _nt(q, k)
            ps = []
            for i in range(WS):
                si = s[i * 8:(i + 1) * 8]
                ma = jnp.max(jnp.where(oka, si, NEG), axis=1, keepdims=True)
                mb = jnp.max(jnp.where(okb, si, NEG), axis=1, keepdims=True)
                ps.append(jnp.exp2(jnp.where(key_ok, si - jnp.where(seg_a, ma, mb), NEG)))
            o = _nn(jnp.concatenate(ps, axis=0).astype(BF16), v)
            for i in range(WS):
                att_s[t, pl.ds(i * WP + c * WS, 8), :] = o[i * 8:(i + 1) * 8]

    l128 = jax.lax.broadcasted_iota(jnp.int32, (8, 128), 1)
    idx01 = jnp.where(l128 < 48, 96, 112)
    idx23 = jnp.where(l128 < 64, 32, 80)

    def stage_c(x0_s, att_s, i, t):
        rows = pl.ds(pl.multiple_of(i * WP + t * 128, 128), 128)
        parts = []
        for j, idx in enumerate((idx01, idx23)):
            a = att_s[j, rows, :]
            pieces = []
            for u in range(16):
                au = a[u * 8:(u + 1) * 8]
                pieces.append(au * pl.reciprocal(jnp.take_along_axis(au, idx, axis=1), approx=True))
            parts.append(jnp.concatenate(pieces, axis=0))
        o = jnp.concatenate(parts, axis=1).astype(BF16)
        y = _nt(wo_s[...], o)
        x0 = x0_s[slot(r - 3) * (WS * 4) + i * 4 + t]
        o_ref[i, :, pl.ds(pl.multiple_of(t * 128, 128), 128)] = (y + x0).astype(o_ref.dtype)

    ORDER = os.environ.get('ORDER', 'seq')

    def step(x0_w, x0_r, qkv_w, qkv_r, att_w, att_r):
        def body(n, carry):
            wins = [jnp.minimum(n * NWI + u, NW - 1) for u in range(NWI)]
            if ORDER == 'seq':
                for tt in range(NT):
                    for i in range(WS):
                        stage_c(x0_r, att_r, i, n * NT + tt)
                for c in wins:
                    stage_b(qkv_r, att_w, c)
                for tt in range(NT):
                    for i in range(WS):
                        stage_l(x0_r, qkv_w, i, n * NT + tt)
                for k in range(NG):
                    stage_a(x0_w, n * NG + k)
            else:
                units = NT * WS
                wi = 0
                gi = 0
                for u in range(units):
                    i, tt = u % WS, u // WS
                    stage_l(x0_r, qkv_w, i, n * NT + tt)
                    we = (u + 1) * NWI // units
                    for c in wins[wi:we]:
                        stage_b(qkv_r, att_w, c)
                    wi = we
                    stage_c(x0_r, att_r, i, n * NT + tt)
                    ge = (u + 1) * NG // units
                    for k in range(gi, ge):
                        stage_a(x0_w, n * NG + k)
                    gi = ge
            return carry
        jax.lax.fori_loop(0, NI, body, 0)

    @pl.when(r % 2 == 0)
    def _even():
        step(x0_e, x0_o, qkv_o, qkv_e, att_e, att_o)

    @pl.when(r % 2 == 1)
    def _odd():
        step(x0_o, x0_e, qkv_e, qkv_o, att_o, att_e)


@jax.jit
def pallas_standalone__window_attn_davit__vision_kernel(
    x: jax.Array,
    dw_pe: jax.Array,
    w_qkv: jax.Array,
    w_o: jax.Array,
):
    xt = jnp.transpose(x.reshape(H, W, C), (0, 2, 1))
    dwt = jnp.transpose(dw_pe.reshape(9, C), (1, 0))
    full = lambda shape: pl.BlockSpec(shape, lambda r: (0,) * len(shape))
    out = pl.pallas_call(
        _kernel,
        grid=(NW + 3,),
        in_specs=[
            pl.BlockSpec((1, C, WP), lambda r: (jnp.maximum(jnp.minimum(r, NW - 1) * WS - 1, 0), 0, 0)),
            pl.BlockSpec((WS, C, WP), lambda r: (jnp.minimum(r, NW - 1), 0, 0)),
            pl.BlockSpec((1, C, WP), lambda r: (jnp.minimum(r * WS + WS, H - 1), 0, 0)),
            full((C, 9)),
            full((C, 3 * C)),
            full((C, C)),
        ],
        out_specs=pl.BlockSpec((WS, C, WP), lambda r: (jnp.maximum(r - 3, 0), 0, 0)),
        out_shape=jax.ShapeDtypeStruct((H, C, W), x.dtype),
        scratch_shapes=[
            pltpu.VMEM((C, 640), BF16),
            pltpu.VMEM((C, 256), BF16),
            pltpu.VMEM((9, C, 128), F32),
            pltpu.VMEM((2 * WS * 4, C, 128), F32),
            pltpu.VMEM((2 * WS * 4, C, 128), F32),
            pltpu.VMEM((5, WS * WP, 128), F32),
            pltpu.VMEM((5, WS * WP, 128), F32),
            pltpu.VMEM((2, WS * WP, 128), F32),
            pltpu.VMEM((2, WS * WP, 128), F32),
        ],
        compiler_params=pltpu.CompilerParams(
            dimension_semantics=("arbitrary",),
            vmem_limit_bytes=64 * 1024 * 1024,
        ),
    )(xt, xt, xt, dwt, w_qkv, w_o)
    return jnp.transpose(out, (0, 2, 1)).reshape(1, H, W, C)
```

```python
import functools
import os
import numpy as np
import jax
import jax.numpy as jnp
import jax.experimental.pallas as pl
import jax.experimental.pallas.tpu as pltpu

WS = 7
NH = 4
C = 192
DH = C // NH
H = W = 511
WP = 512
NW = W // WS
EPS = 1e-05
NEG = -1e30
F32 = jnp.float32
BF16 = jnp.bfloat16


def _nt(a, b):
    return jax.lax.dot_general(a, b, (((1,), (1,)), ((), ())), preferred_element_type=F32)


def _nn(a, b):
    return jax.lax.dot_general(a, b, (((1,), (0,)), ((), ())), preferred_element_type=F32)


def _kernel(xt_ref, xm_ref, xb_ref, dw_ref, wqkv_ref, wo_ref, o_ref,
            wq_s, wo_s, dwb_s, x0_e, x0_o, qkv_e, qkv_o, att_e, att_o):
    r = pl.program_id(0)

    @pl.when(r == 0)
    def _prep():
        w = wqkv_ref[...].astype(F32)
        qs = w[:, 0:C] * np.float32(DH ** -0.5 * np.log2(np.e))
        q = [qs[:, h * DH:(h + 1) * DH] for h in range(NH)]
        k = [w[:, C + h * DH:C + (h + 1) * DH] for h in range(NH)]
        v = [w[:, 2 * C + h * DH:2 * C + (h + 1) * DH] for h in range(NH)]
        z32 = jnp.zeros((C, 32), F32)
        tiles = [
            [q[0], v[2][:, 32:48], v[3][:, 0:16], q[1]],
            [v[2][:, 0:32], q[2], q[3]],
            [k[0], z32, k[1]],
            [z32, k[2], k[3]],
            [v[0], v[1], v[3][:, 16:48]],
        ]
        for t in range(5):
            wq_s[:, t * 128:(t + 1) * 128] = jnp.concatenate(tiles[t], axis=1).astype(BF16)
        wo = wo_ref[...].astype(F32)
        zr = lambda n: jnp.zeros((n, C), F32)
        wo2 = jnp.concatenate([
            wo[0:96], zr(32),
            wo[96:128], zr(16), wo[128:144], wo[144:160], zr(16), wo[160:192]], axis=0)
        wo_s[...] = wo2.T.astype(BF16)
        dw = dw_ref[...].astype(F32)
        for j in range(9):
            col = dw[:, j:j + 1]
            if j == 4:
                col = col + 1.0
            dwb_s[j] = jnp.broadcast_to(col, (C, 128))

        x0_e[...] = jnp.zeros(x0_e.shape, F32)
        x0_o[...] = jnp.zeros(x0_o.shape, F32)
        qkv_e[...] = jnp.zeros(qkv_e.shape, F32)
        att_o[...] = jnp.ones(att_o.shape, F32)

    NI = int(os.environ.get('NI', '2'))
    NT = 4 // NI
    NG = 12 // NI
    NWI = -(-NW // NI)
    lane16 = jax.lax.broadcasted_iota(jnp.int32, (16, 128), 1)
    l8 = jax.lax.broadcasted_iota(jnp.int32, (8, 128), 1)
    seg_a = l8 < 64
    key_ok = jnp.logical_and((l8 % 64) < 56, (l8 % 8) < 7)
    oka = jnp.logical_and(key_ok, seg_a)
    okb = jnp.logical_and(key_ok, jnp.logical_not(seg_a))
    ra = jnp.minimum(r, NW - 1)
    top_ok = ra > 0
    bot_ok = ra < NW - 1

    def between(lo, hi):
        return jnp.logical_and(l8 >= lo, l8 < hi)

    def ones_at(lo, hi):
        return jnp.where(between(lo, hi), 1.0, 0.0).astype(F32)

    def slot(q):
        return ((q + 4) // 2) % 2

    def stage_a(x0_s, g, half=None):
        cs = pl.ds(pl.multiple_of(g * 16, 16), 16)
        base = slot(r) * (WS * 4)
        if half is None:
            co, lane_a = cs, lane16
        else:
            co, lane_a = pl.ds(pl.multiple_of(g * 16 + half * 8, 8), 8), l8
        wts = [dwb_s[j, co, :] for j in range(9)]

        def load_row(i):
            if i == -1:
                v = jnp.where(top_ok, xt_ref[0, cs, :].astype(F32), 0.0)
            elif i == WS:
                v = jnp.where(bot_ok, xb_ref[0, cs, :].astype(F32), 0.0)
            else:
                v = xm_ref[i, cs, :].astype(F32)
            if half is not None:
                v = v[half * 8:(half + 1) * 8]
            parts = [v[:, t * 128:(t + 1) * 128] for t in range(4)]
            parts[3] = jnp.where(lane16[:v.shape[0]] < 127, parts[3], 0.0)
            return parts

        rows = {-1: load_row(-1), 0: load_row(0)}
        for i in range(WS):
            rows[i + 1] = load_row(i + 1)
            v0, v1, v2 = [], [], []
            for t in range(4):
                a, b, c = rows[i - 1][t], rows[i][t], rows[i + 1][t]
                v0.append(pltpu.roll(a * wts[0] + b * wts[3] + c * wts[6], 1, 1))
                v1.append(a * wts[1] + b * wts[4] + c * wts[7])
                v2.append(pltpu.roll(a * wts[2] + b * wts[5] + c * wts[8], 127, 1))
            for t in range(4):
                l = jnp.where(lane_a == 0, 0.0 if t == 0 else v0[t - 1], v0[t])
                rr = jnp.where(lane_a == 127, 0.0 if t == 3 else v2[t + 1], v2[t])
                x0_s[base + (i * 4 + t), co, :] = v1[t] + l + rr
            del rows[i - 1]

    def stage_l(x0_s, qkv_s, i, t):
        x0 = x0_s[slot(r - 1) * (WS * 4) + i * 4 + t]
        m = jnp.mean(x0, axis=0, keepdims=True)
        d = x0 - m
        var = jnp.mean(d * d, axis=0, keepdims=True)
        h = d * jax.lax.rsqrt(var + EPS)
        ht = h.T.astype(BF16)
        qkv = _nn(ht, wq_s[...])
        rows = pl.ds(pl.multiple_of(i * WP + t * 128, 128), 128)
        for j in range(5):
            qkv_s[j, rows, :] = qkv[:, j * 128:(j + 1) * 128]

    z8 = jnp.zeros((8, 128), F32)

    def ext(rows_a, rows_b):
        return jnp.concatenate(rows_a + [z8] + rows_b + [z8], axis=0).astype(BF16)

    def stage_b1(qkv_s, c):
        def ld(t):
            return [qkv_s[t, pl.ds(i * WP + c * WS, 8), :] for i in range(WS)]

        t2, t3 = ld(2), ld(3)
        k01 = ext([jnp.where(l8 < 48, x, 0.0) for x in t2], [jnp.where(l8 >= 80, x, 0.0) for x in t2])
        k23 = ext([jnp.where(between(32, 80), x, 0.0) for x in t3], [jnp.where(l8 >= 80, x, 0.0) for x in t3])
        q01 = jnp.concatenate(ld(0), axis=0).astype(BF16)
        q23 = jnp.concatenate(ld(1), axis=0).astype(BF16)
        return _nt(q01, k01), _nt(q23, k23)

    def stage_b2(qkv_s, att_s, c, ss):
        def ld(t):
            return [qkv_s[t, pl.ds(i * WP + c * WS, 8), :] for i in range(WS)]

        for t, s in enumerate(ss):
            ps = []
            for i in range(WS):
                si = s[i * 8:(i + 1) * 8]
                ma = jnp.max(jnp.where(oka, si, NEG), axis=1, keepdims=True)
                mb = jnp.max(jnp.where(okb, si, NEG), axis=1, keepdims=True)
                ps.append(jnp.exp2(jnp.where(key_ok, si - jnp.where(seg_a, ma, mb), NEG)))
            if t == 0:
                t4 = ld(4)
                v = ext([jnp.where(l8 < 48, x, ones_at(96, 112)) for x in t4],
                        [jnp.where(between(48, 96), x, ones_at(112, 128)) for x in t4])
            else:
                t0, t1, t4 = ld(0), ld(1), ld(4)
                v = ext([jnp.where(l8 < 32, b, jnp.where(between(48, 64), a, ones_at(32, 48))) for a, b in zip(t0, t1)],
                        [jnp.where(l8 >= 96, d, jnp.where(between(64, 80), a, ones_at(80, 96))) for a, d in zip(t0, t4)])
            o = _nn(jnp.concatenate(ps, axis=0).astype(BF16), v)
            for i in range(WS):
                att_s[t, pl.ds(i * WP + c * WS, 8), :] = o[i * 8:(i + 1) * 8]

    def b_items(qkv_s, att_s, wins, lag):
        pend = {}

        def f1(u):
            pend[u] = stage_b1(qkv_s, wins[u])

        def f2(u):
            stage_b2(qkv_s, att_s, wins[u], pend.pop(u))

        items = []
        for u in range(len(wins) + lag):
            if u < len(wins):
                items.append(functools.partial(f1, u))
            if u >= lag:
                items.append(functools.partial(f2, u - lag))
        return items

    l128 = jax.lax.broadcasted_iota(jnp.int32, (8, 128), 1)
    idx01 = jnp.where(l128 < 48, 96, 112)
    idx23 = jnp.where(l128 < 64, 32, 80)

    def stage_c(x0_s, att_s, i, t):
        rows = pl.ds(pl.multiple_of(i * WP + t * 128, 128), 128)
        parts = []
        for j, idx in enumerate((idx01, idx23)):
            a = att_s[j, rows, :]
            pieces = []
            for u in range(16):
                au = a[u * 8:(u + 1) * 8]
                pieces.append(au * pl.reciprocal(jnp.take_along_axis(au, idx, axis=1), approx=True))
            parts.append(jnp.concatenate(pieces, axis=0))
        o = jnp.concatenate(parts, axis=1).astype(BF16)
        y = _nt(wo_s[...], o)
        x0 = x0_s[slot(r - 3) * (WS * 4) + i * 4 + t]
        o_ref[i, :, pl.ds(pl.multiple_of(t * 128, 128), 128)] = (y + x0).astype(o_ref.dtype)

    ORDER = os.environ.get('ORDER', 'B,LA,C')

    def step(x0_w, x0_r, qkv_w, qkv_r, att_w, att_r):
        def body(n, carry):
            wins = [jnp.minimum(n * NWI + u, NW - 1) for u in range(NWI)]
            items = {
                'C': [functools.partial(stage_c, x0_r, att_r, u % WS, n * NT + u // WS) for u in range(NT * WS)],
                'B': b_items(qkv_r, att_w, wins, int(os.environ.get('BLAG', '1'))),
                'L': [functools.partial(stage_l, x0_r, qkv_w, u % WS, n * NT + u // WS) for u in range(NT * WS)],
                'A': ([functools.partial(stage_a, x0_w, n * NG + k) for k in range(NG)] if os.environ.get('AHALF', '1') == '0' else
                      [functools.partial(stage_a, x0_w, n * NG + k, hf) for k in range(NG) for hf in range(2)]),
            }
            for group in ORDER.split(','):
                n_steps = max(len(items[s]) for s in group)
                pos = {s: 0 for s in group}
                for u in range(n_steps):
                    for s in group:
                        e = -(-(u + 1) * len(items[s]) // n_steps)
                        for f in items[s][pos[s]:e]:
                            f()
                        pos[s] = e
            return carry
        jax.lax.fori_loop(0, NI, body, 0)

    @pl.when(r % 2 == 0)
    def _even():
        step(x0_e, x0_o, qkv_o, qkv_e, att_e, att_o)

    @pl.when(r % 2 == 1)
    def _odd():
        step(x0_o, x0_e, qkv_e, qkv_o, att_o, att_e)


@jax.jit
def pallas_standalone__window_attn_davit__vision_kernel(
    x: jax.Array,
    dw_pe: jax.Array,
    w_qkv: jax.Array,
    w_o: jax.Array,
):
    xt = jnp.transpose(x.reshape(H, W, C), (0, 2, 1))
    dwt = jnp.transpose(dw_pe.reshape(9, C), (1, 0))
    full = lambda shape: pl.BlockSpec(shape, lambda r: (0,) * len(shape))
    out = pl.pallas_call(
        _kernel,
        grid=(NW + 3,),
        in_specs=[
            pl.BlockSpec((1, C, WP), lambda r: (jnp.maximum(jnp.minimum(r, NW - 1) * WS - 1, 0), 0, 0)),
            pl.BlockSpec((WS, C, WP), lambda r: (jnp.minimum(r, NW - 1), 0, 0)),
            pl.BlockSpec((1, C, WP), lambda r: (jnp.minimum(r * WS + WS, H - 1), 0, 0)),
            full((C, 9)),
            full((C, 3 * C)),
            full((C, C)),
        ],
        out_specs=pl.BlockSpec((WS, C, WP), lambda r: (jnp.maximum(r - 3, 0), 0, 0)),
        out_shape=jax.ShapeDtypeStruct((H, C, W), x.dtype),
        scratch_shapes=[
            pltpu.VMEM((C, 640), BF16),
            pltpu.VMEM((C, 256), BF16),
            pltpu.VMEM((9, C, 128), F32),
            pltpu.VMEM((2 * WS * 4, C, 128), F32),
            pltpu.VMEM((2 * WS * 4, C, 128), F32),
            pltpu.VMEM((5, WS * WP, 128), F32),
            pltpu.VMEM((5, WS * WP, 128), F32),
            pltpu.VMEM((2, WS * WP, 128), F32),
            pltpu.VMEM((2, WS * WP, 128), F32),
        ],
        compiler_params=pltpu.CompilerParams(
            dimension_semantics=("arbitrary",),
            vmem_limit_bytes=64 * 1024 * 1024,
            flags={k: True for k in os.environ.get('KFLAGS', '').split(',') if k},
        ),
    )(xt, xt, xt, dwt, w_qkv, w_o)
    return jnp.transpose(out, (0, 2, 1)).reshape(1, H, W, C)
```

```python
import functools
import os
import numpy as np
import jax
import jax.numpy as jnp
import jax.experimental.pallas as pl
import jax.experimental.pallas.tpu as pltpu

WS = 7
NH = 4
C = 192
DH = C // NH
H = W = 511
WP = 512
NW = W // WS
NSTEP = NW + 3
EPS = 1e-05
NEG = -1e30
F32 = jnp.float32
BF16 = jnp.bfloat16
BLAG = int(os.environ.get('BLAG', '1'))
ORDER = os.environ.get('ORDER', 'B,AL,C')


def _nt(a, b):
    return jax.lax.dot_general(a, b, (((1,), (1,)), ((), ())), preferred_element_type=F32)


def _nn(a, b):
    return jax.lax.dot_general(a, b, (((1,), (0,)), ((), ())), preferred_element_type=F32)


def _kernel(xt_ref, xm_ref, xb_ref, dw_ref, wqkv_ref, wo_ref, o_ref,
            wq_s, wo_s, dwb_s, x0_e, x0_o, qkv_e, qkv_o, att_e, att_o):
    lane16 = jax.lax.broadcasted_iota(jnp.int32, (16, 128), 1)
    l8 = jax.lax.broadcasted_iota(jnp.int32, (8, 128), 1)
    seg_a = l8 < 64
    key_ok = jnp.logical_and((l8 % 64) < 56, (l8 % 8) < 7)
    oka = jnp.logical_and(key_ok, seg_a)
    okb = jnp.logical_and(key_ok, jnp.logical_not(seg_a))
    z8 = jnp.zeros((8, 128), F32)

    def between(lo, hi):
        return jnp.logical_and(l8 >= lo, l8 < hi)

    def ones_at(lo, hi):
        return jnp.where(between(lo, hi), 1.0, 0.0).astype(F32)

    def slot(q):
        return ((q + 4) // 2) % 2

    def prepare_weights():
        w = wqkv_ref[...].astype(F32)
        qs = w[:, 0:C] * np.float32(DH ** -0.5 * np.log2(np.e))
        q = [qs[:, h * DH:(h + 1) * DH] for h in range(NH)]
        k = [w[:, C + h * DH:C + (h + 1) * DH] for h in range(NH)]
        v = [w[:, 2 * C + h * DH:2 * C + (h + 1) * DH] for h in range(NH)]
        z32 = jnp.zeros((C, 32), F32)
        tiles = [
            [q[0], v[2][:, 32:48], v[3][:, 0:16], q[1]],
            [v[2][:, 0:32], q[2], q[3]],
            [k[0], z32, k[1]],
            [z32, k[2], k[3]],
            [v[0], v[1], v[3][:, 16:48]],
        ]
        for t in range(5):
            wq_s[:, t * 128:(t + 1) * 128] = jnp.concatenate(tiles[t], axis=1).astype(BF16)
        wo = wo_ref[...].astype(F32)
        zr = lambda n: jnp.zeros((n, C), F32)
        wo2 = jnp.concatenate([wo[0:96], zr(32), wo[96:128], zr(16), wo[128:160], zr(16), wo[160:192]], axis=0)
        wo_s[...] = wo2.T.astype(BF16)
        dw = dw_ref[...].astype(F32)
        for j in range(9):
            col = dw[:, j:j + 1]
            if j == 4:
                col = col + 1.0
            dwb_s[j] = jnp.broadcast_to(col, (C, 128))

    def stage_a(r, x0_s, g, half):
        cs = pl.ds(g * 16, 16)
        co = pl.ds(g * 16 + half * 8, 8)
        base = slot(r) * (WS * 4)
        wts = [dwb_s[j, co, :] for j in range(9)]
        ra = min(r, NW - 1) if isinstance(r, int) else jnp.minimum(r, NW - 1)

        def load_row(i):
            if i == -1:
                v = jnp.where(ra > 0, xt_ref[0, cs, :].astype(F32), 0.0)
            elif i == WS:
                v = jnp.where(ra < NW - 1, xb_ref[0, cs, :].astype(F32), 0.0)
            else:
                v = xm_ref[i, cs, :].astype(F32)
            v = v[half * 8:(half + 1) * 8]
            parts = [v[:, t * 128:(t + 1) * 128] for t in range(4)]
            parts[3] = jnp.where(l8 < W - 3 * 128, parts[3], 0.0)
            return parts

        rows = {-1: load_row(-1), 0: load_row(0)}
        for i in range(WS):
            rows[i + 1] = load_row(i + 1)
            v0, v1, v2 = [], [], []
            for t in range(4):
                a, b, c = rows[i - 1][t], rows[i][t], rows[i + 1][t]
                v0.append(pltpu.roll(a * wts[0] + b * wts[3] + c * wts[6], 1, 1))
                v1.append(a * wts[1] + b * wts[4] + c * wts[7])
                v2.append(pltpu.roll(a * wts[2] + b * wts[5] + c * wts[8], 127, 1))
            for t in range(4):
                lf = jnp.where(l8 == 0, 0.0 if t == 0 else v0[t - 1], v0[t])
                rt = jnp.where(l8 == 127, 0.0 if t == 3 else v2[t + 1], v2[t])
                x0_s[base + (i * 4 + t), co, :] = v1[t] + lf + rt
            del rows[i - 1]

    def stage_l(r, x0_s, qkv_s, i, t):
        x0 = x0_s[slot(r - 1) * (WS * 4) + i * 4 + t]
        m = jnp.mean(x0, axis=0, keepdims=True)
        d = x0 - m
        var = jnp.mean(d * d, axis=0, keepdims=True)
        h = d * jax.lax.rsqrt(var + EPS)
        qkv = _nn(h.T.astype(BF16), wq_s[...])
        for j in range(5):
            qkv_s[j, pl.ds(i * WP + t * 128, 128), :] = qkv[:, j * 128:(j + 1) * 128]

    def ext(rows_a, rows_b):
        return jnp.concatenate(rows_a + [z8] + rows_b + [z8], axis=0).astype(BF16)

    def ld(qkv_s, t, c):
        return [qkv_s[t, pl.ds(i * WP + c * WS, 8), :] for i in range(WS)]

    def stage_b1(qkv_s, c):
        t2, t3 = ld(qkv_s, 2, c), ld(qkv_s, 3, c)
        k01 = ext([jnp.where(l8 < 48, x, 0.0) for x in t2], [jnp.where(l8 >= 80, x, 0.0) for x in t2])
        k23 = ext([jnp.where(between(32, 80), x, 0.0) for x in t3], [jnp.where(l8 >= 80, x, 0.0) for x in t3])
        q01 = jnp.concatenate(ld(qkv_s, 0, c), axis=0).astype(BF16)
        q23 = jnp.concatenate(ld(qkv_s, 1, c), axis=0).astype(BF16)
        return _nt(q01, k01), _nt(q23, k23)

    def stage_b2(qkv_s, att_s, c, ss):
        for t, s in enumerate(ss):
            ps = []
            for i in range(WS):
                si = s[i * 8:(i + 1) * 8]
                ma = jnp.max(jnp.where(oka, si, NEG), axis=1, keepdims=True)
                mb = jnp.max(jnp.where(okb, si, NEG), axis=1, keepdims=True)
                ps.append(jnp.exp2(jnp.where(key_ok, si - jnp.where(seg_a, ma, mb), NEG)))
            if t == 0:
                t4 = ld(qkv_s, 4, c)
                v = ext([jnp.where(l8 < 48, x, ones_at(96, 112)) for x in t4],
                        [jnp.where(between(48, 96), x, ones_at(112, 128)) for x in t4])
            else:
                t0, t1, t4 = ld(qkv_s, 0, c), ld(qkv_s, 1, c), ld(qkv_s, 4, c)
                v = ext([jnp.where(l8 < 32, b, jnp.where(between(48, 64), a, ones_at(32, 48))) for a, b in zip(t0, t1)],
                        [jnp.where(l8 >= 96, d, jnp.where(between(64, 80), a, ones_at(80, 96))) for a, d in zip(t0, t4)])
            o = _nn(jnp.concatenate(ps, axis=0).astype(BF16), v)
            for i in range(WS):
                att_s[t, pl.ds(i * WP + c * WS, 8), :] = o[i * 8:(i + 1) * 8]

    def b_items(qkv_s, att_s):
        pend = {}

        def f1(c):
            pend[c] = stage_b1(qkv_s, c)

        def f2(c):
            stage_b2(qkv_s, att_s, c, pend.pop(c))

        items = []
        for u in range(NW + BLAG):
            if u < NW:
                items.append(functools.partial(f1, u))
            if u >= BLAG:
                items.append(functools.partial(f2, u - BLAG))
        return items

    idx01 = jnp.where(l8 < 48, 96, 112)
    idx23 = jnp.where(l8 < 64, 32, 80)

    def stage_c(r, x0_s, att_s, i, t):
        parts = []
        for j, idx in enumerate((idx01, idx23)):
            a = att_s[j, pl.ds(i * WP + t * 128, 128), :]
            pieces = []
            for u in range(16):
                au = a[u * 8:(u + 1) * 8]
                pieces.append(au * pl.reciprocal(jnp.take_along_axis(au, idx, axis=1), approx=True))
            parts.append(jnp.concatenate(pieces, axis=0))
        o = jnp.concatenate(parts, axis=1).astype(BF16)
        y = _nt(wo_s[...], o)
        x0 = x0_s[slot(r - 3) * (WS * 4) + i * 4 + t]
        o_ref[i, :, t * 128:(t + 1) * 128] = (y + x0).astype(o_ref.dtype)

    def step(r, parity, stages, extra=()):
        x0_w, x0_r, qkv_w, qkv_r, att_w, att_r = (
            (x0_e, x0_o, qkv_o, qkv_e, att_e, att_o) if parity == 0 else (x0_o, x0_e, qkv_e, qkv_o, att_o, att_e))
        units = [(u % WS, u // WS) for u in range(4 * WS)]
        items = {
            'A': [functools.partial(stage_a, r, x0_w, g, hf) for g in range(C // 16) for hf in range(2)],
            'L': [functools.partial(stage_l, r, x0_r, qkv_w, i, t) for i, t in units],
            'B': b_items(qkv_r, att_w),
            'C': [functools.partial(stage_c, r, x0_r, att_r, i, t) for i, t in units],
            'X': list(extra),
        }
        for group in ORDER.split(','):
            names = [s for s in group if s in stages]
            if not names:
                continue
            n_steps = max(len(items[s]) for s in names)
            pos = {s: 0 for s in names}
            for u in range(n_steps):
                for s in names:
                    e = -(-(u + 1) * len(items[s]) // n_steps)
                    for f in items[s][pos[s]:e]:
                        f()
                    pos[s] = e

    r = pl.program_id(0)

    @pl.when(r == 0)
    def _first():
        prepare_weights()
        att_o[...] = jnp.ones(att_o.shape, F32)
        x0_o[pl.ds(slot(-1) * WS * 4, WS * 4)] = jnp.zeros((WS * 4, C, 128), F32)
        step(0, 0, 'A')

    @pl.when(r == 1)
    def _second():
        step(1, 1, 'AL')

    @pl.when(jnp.logical_and(r % 2 == 0, jnp.logical_and(r >= 2, r <= NW - 1)))
    def _even():
        step(r, 0, 'ABCL')

    @pl.when(jnp.logical_and(r % 2 == 1, jnp.logical_and(r >= 2, r <= NW)))
    def _odd():
        step(r, 1, 'ABCL')

    @pl.when(r == NW + 1)
    def _second_last():
        step(NW + 1, (NW + 1) % 2, 'BC')

    @pl.when(r == NW + 2)
    def _last():
        step(NW + 2, (NW + 2) % 2, 'C')


@jax.jit
def pallas_standalone__window_attn_davit__vision_kernel(
    x: jax.Array,
    dw_pe: jax.Array,
    w_qkv: jax.Array,
    w_o: jax.Array,
):
    xt = jnp.transpose(x.reshape(H, W, C), (0, 2, 1))
    dwt = jnp.transpose(dw_pe.reshape(9, C), (1, 0))
    full = lambda shape: pl.BlockSpec(shape, lambda r: (0,) * len(shape))
    out = pl.pallas_call(
        _kernel,
        grid=(NSTEP,),
        in_specs=[
            pl.BlockSpec((1, C, WP), lambda r: (jnp.maximum(jnp.minimum(r, NW - 1) * WS - 1, 0), 0, 0)),
            pl.BlockSpec((WS, C, WP), lambda r: (jnp.minimum(r, NW - 1), 0, 0)),
            pl.BlockSpec((1, C, WP), lambda r: (jnp.minimum(r * WS + WS, H - 1), 0, 0)),
            full((C, 9)),
            full((C, 3 * C)),
            full((C, C)),
        ],
        out_specs=pl.BlockSpec((WS, C, WP), lambda r: (jnp.maximum(r - 3, 0), 0, 0)),
        out_shape=jax.ShapeDtypeStruct((H, C, W), x.dtype),
        scratch_shapes=[
            pltpu.VMEM((C, 640), BF16),
            pltpu.VMEM((C, 256), BF16),
            pltpu.VMEM((9, C, 128), F32),
            pltpu.VMEM((2 * WS * 4, C, 128), F32),
            pltpu.VMEM((2 * WS * 4, C, 128), F32),
            pltpu.VMEM((5, WS * WP, 128), F32),
            pltpu.VMEM((5, WS * WP, 128), F32),
            pltpu.VMEM((2, WS * WP, 128), F32),
            pltpu.VMEM((2, WS * WP, 128), F32),
        ],
        compiler_params=pltpu.CompilerParams(
            dimension_semantics=("arbitrary",),
            vmem_limit_bytes=64 * 1024 * 1024,
        ),
    )(xt, xt, xt, dwt, w_qkv, w_o)
    return jnp.transpose(out, (0, 2, 1)).reshape(1, H, W, C)
```

```python
import functools
import os
import re
import numpy as np
import jax
import jax.numpy as jnp
import jax.experimental.pallas as pl
import jax.experimental.pallas.tpu as pltpu

WS = 7
NH = 4
C = 192
DH = C // NH
H = W = 511
WP = 512
NW = W // WS
NSTEP = NW + 3
EPS = 1e-05
NEG = -1e30
F32 = jnp.float32
BF16 = jnp.bfloat16
BLAG = int(os.environ.get('BLAG', '1'))
ORDER = os.environ.get('ORDER', 'B,AL,C')


def _nt(a, b):
    return jax.lax.dot_general(a, b, (((1,), (1,)), ((), ())), preferred_element_type=F32)


def _nn(a, b):
    return jax.lax.dot_general(a, b, (((1,), (0,)), ((), ())), preferred_element_type=F32)


def _kernel(xt_ref, xm_ref, xb_ref, dw_ref, wqkv_ref, wo_ref, o_ref,
            wq_s, wo_s, dwb_s, x0_e, x0_o, qkv_e, qkv_o, att_e, att_o):
    lane16 = jax.lax.broadcasted_iota(jnp.int32, (16, 128), 1)
    l8 = jax.lax.broadcasted_iota(jnp.int32, (8, 128), 1)
    seg_a = l8 < 64
    key_ok = jnp.logical_and((l8 % 64) < 56, (l8 % 8) < 7)
    oka = jnp.logical_and(key_ok, seg_a)
    okb = jnp.logical_and(key_ok, jnp.logical_not(seg_a))
    z8 = jnp.zeros((8, 128), F32)

    def between(lo, hi):
        return jnp.logical_and(l8 >= lo, l8 < hi)

    def ones_at(lo, hi):
        return jnp.where(between(lo, hi), 1.0, 0.0).astype(F32)

    def slot(q):
        return ((q + 4) // 2) % 2

    def prepare_weights():
        w = wqkv_ref[...].astype(F32)
        qs = w[:, 0:C] * np.float32(DH ** -0.5 * np.log2(np.e))
        q = [qs[:, h * DH:(h + 1) * DH] for h in range(NH)]
        k = [w[:, C + h * DH:C + (h + 1) * DH] for h in range(NH)]
        v = [w[:, 2 * C + h * DH:2 * C + (h + 1) * DH] for h in range(NH)]
        z32 = jnp.zeros((C, 32), F32)
        tiles = [
            [q[0], v[2][:, 32:48], v[3][:, 0:16], q[1]],
            [v[2][:, 0:32], q[2], q[3]],
            [k[0], z32, k[1]],
            [z32, k[2], k[3]],
            [v[0], v[1], v[3][:, 16:48]],
        ]
        for t in range(5):
            wq_s[:, t * 128:(t + 1) * 128] = jnp.concatenate(tiles[t], axis=1).astype(BF16)
        wo = wo_ref[...].astype(F32)
        zr = lambda n: jnp.zeros((n, C), F32)
        wo2 = jnp.concatenate([wo[0:96], zr(32), wo[96:128], zr(16), wo[128:160], zr(16), wo[160:192]], axis=0)
        wo_s[...] = wo2.T.astype(BF16)
        dw = dw_ref[...].astype(F32)
        for j in range(9):
            col = dw[:, j:j + 1]
            if j == 4:
                col = col + 1.0
            dwb_s[j] = jnp.broadcast_to(col, (C, 128))

    def stage_a(r, x0_s, g, half):
        cs = pl.ds(g * 16, 16)
        co = pl.ds(g * 16 + half * 8, 8)
        base = slot(r) * (WS * 4)
        wts = [dwb_s[j, co, :] for j in range(9)]
        ra = min(r, NW - 1) if isinstance(r, int) else jnp.minimum(r, NW - 1)

        def load_row(i):
            if i == -1:
                v = jnp.where(ra > 0, xt_ref[0, cs, :].astype(F32), 0.0)
            elif i == WS:
                v = jnp.where(ra < NW - 1, xb_ref[0, cs, :].astype(F32), 0.0)
            else:
                v = xm_ref[i, cs, :].astype(F32)
            v = v[half * 8:(half + 1) * 8]
            parts = [v[:, t * 128:(t + 1) * 128] for t in range(4)]
            parts[3] = jnp.where(l8 < W - 3 * 128, parts[3], 0.0)
            return parts

        rows = {-1: load_row(-1), 0: load_row(0)}
        for i in range(WS):
            rows[i + 1] = load_row(i + 1)
            v0, v1, v2 = [], [], []
            for t in range(4):
                a, b, c = rows[i - 1][t], rows[i][t], rows[i + 1][t]
                v0.append(pltpu.roll(a * wts[0] + b * wts[3] + c * wts[6], 1, 1))
                v1.append(a * wts[1] + b * wts[4] + c * wts[7])
                v2.append(pltpu.roll(a * wts[2] + b * wts[5] + c * wts[8], 127, 1))
            for t in range(4):
                lf = jnp.where(l8 == 0, 0.0 if t == 0 else v0[t - 1], v0[t])
                rt = jnp.where(l8 == 127, 0.0 if t == 3 else v2[t + 1], v2[t])
                x0_s[base + (i * 4 + t), co, :] = v1[t] + lf + rt
            del rows[i - 1]

    def stage_l(r, x0_s, qkv_s, i, t):
        x0 = x0_s[slot(r - 1) * (WS * 4) + i * 4 + t]
        m = jnp.mean(x0, axis=0, keepdims=True)
        d = x0 - m
        var = jnp.mean(d * d, axis=0, keepdims=True)
        h = d * jax.lax.rsqrt(var + EPS)
        qkv = _nn(h.T.astype(BF16), wq_s[...])
        for j in range(5):
            qkv_s[j, pl.ds(i * WP + t * 128, 128), :] = qkv[:, j * 128:(j + 1) * 128]

    def ext(rows_a, rows_b):
        return jnp.concatenate(rows_a + [z8] + rows_b + [z8], axis=0).astype(BF16)

    def ld(qkv_s, t, c):
        return [qkv_s[t, pl.ds(i * WP + c * WS, 8), :] for i in range(WS)]

    def stage_b1(qkv_s, c):
        t2, t3 = ld(qkv_s, 2, c), ld(qkv_s, 3, c)
        k01 = ext([jnp.where(l8 < 48, x, 0.0) for x in t2], [jnp.where(l8 >= 80, x, 0.0) for x in t2])
        k23 = ext([jnp.where(between(32, 80), x, 0.0) for x in t3], [jnp.where(l8 >= 80, x, 0.0) for x in t3])
        q01 = jnp.concatenate(ld(qkv_s, 0, c), axis=0).astype(BF16)
        q23 = jnp.concatenate(ld(qkv_s, 1, c), axis=0).astype(BF16)
        return _nt(q01, k01), _nt(q23, k23)

    def stage_b2(qkv_s, att_s, c, ss, exact):
        outs = []
        for t, s in enumerate(ss):
            ps = []
            for i in range(WS):
                si = s[i * 8:(i + 1) * 8]
                if exact:
                    ma = jnp.max(jnp.where(oka, si, NEG), axis=1, keepdims=True)
                    mb = jnp.max(jnp.where(okb, si, NEG), axis=1, keepdims=True)
                    ps.append(jnp.exp2(jnp.where(key_ok, si - jnp.where(seg_a, ma, mb), NEG)))
                else:
                    sm = jnp.where(key_ok, si, NEG)
                    ps.append(jnp.exp2(sm - jnp.max(sm, axis=1, keepdims=True)))
            if t == 0:
                t4 = ld(qkv_s, 4, c)
                v = ext([jnp.where(l8 < 48, x, ones_at(96, 112)) for x in t4],
                        [jnp.where(between(48, 96), x, ones_at(112, 128)) for x in t4])
            else:
                t0, t1, t4 = ld(qkv_s, 0, c), ld(qkv_s, 1, c), ld(qkv_s, 4, c)
                v = ext([jnp.where(l8 < 32, b, jnp.where(between(48, 64), a, ones_at(32, 48))) for a, b in zip(t0, t1)],
                        [jnp.where(l8 >= 96, d, jnp.where(between(64, 80), a, ones_at(80, 96))) for a, d in zip(t0, t4)])
            o = _nn(jnp.concatenate(ps, axis=0).astype(BF16), v)
            for i in range(WS):
                att_s[t, pl.ds(i * WP + c * WS, 8), :] = o[i * 8:(i + 1) * 8]
            outs.append(o)
        return outs

    def b_items(qkv_s, att_s, low):
        pend = {}

        def f1(c):
            pend[c] = stage_b1(qkv_s, c)

        def f2(c):
            for t, o in enumerate(stage_b2(qkv_s, att_s, c, pend.pop(c), False)):
                for i in range(WS):
                    oi = o[i * 8:(i + 1) * 8]
                    low[t] = oi if low[t] is None else jnp.minimum(low[t], oi)

        items = []
        for u in range(NW + BLAG):
            if u < NW:
                items.append(functools.partial(f1, u))
            if u >= BLAG:
                items.append(functools.partial(f2, u - BLAG))
        return items

    idx01 = jnp.where(l8 < 48, 96, 112)
    idx23 = jnp.where(l8 < 64, 32, 80)

    def stage_c(r, x0_s, att_s, i, t):
        parts = []
        for j, idx in enumerate((idx01, idx23)):
            a = att_s[j, pl.ds(i * WP + t * 128, 128), :]
            pieces = []
            for u in range(16):
                au = a[u * 8:(u + 1) * 8]
                pieces.append(au * pl.reciprocal(jnp.take_along_axis(au, idx, axis=1), approx=True))
            parts.append(jnp.concatenate(pieces, axis=0))
        o = jnp.concatenate(parts, axis=1).astype(BF16)
        y = _nt(wo_s[...], o)
        x0 = x0_s[slot(r - 3) * (WS * 4) + i * 4 + t]
        o_ref[i, :, t * 128:(t + 1) * 128] = (y + x0).astype(o_ref.dtype)

    def step(r, parity, stages, extra=()):
        x0_w, x0_r, qkv_w, qkv_r, att_w, att_r = (
            (x0_e, x0_o, qkv_o, qkv_e, att_e, att_o) if parity == 0 else (x0_o, x0_e, qkv_e, qkv_o, att_o, att_e))
        units = [(u % WS, u // WS) for u in range(4 * WS)]
        low = [None, None]
        items = {
            'A': [functools.partial(stage_a, r, x0_w, g, hf) for g in range(C // 16) for hf in range(2)],
            'L': [functools.partial(stage_l, r, x0_r, qkv_w, i, t) for i, t in units],
            'B': b_items(qkv_r, att_w, low),
            'C': [functools.partial(stage_c, r, x0_r, att_r, i, t) for i, t in units],
            'X': list(extra),
        }
        taken = {s: 0 for s in items}
        for group in ORDER.split(','):
            sel = []
            for s, cnt in re.findall(r'([ABCL])(\d*)', group):
                if s in stages:
                    e = len(items[s]) if not cnt else min(len(items[s]), taken[s] + int(cnt))
                    sel.append(items[s][taken[s]:e])
                    taken[s] = e
            if not sel:
                continue
            n_steps = max(len(q) for q in sel)
            pos = [0] * len(sel)
            for u in range(n_steps):
                for j, q in enumerate(sel):
                    e = -(-(u + 1) * len(q) // n_steps)
                    for f in q[pos[j]:e]:
                        f()
                    pos[j] = e
        for s in stages:
            assert taken[s] == len(items[s])
        if 'B' in stages:
            l01 = jnp.where(l8 >= 96, low[0], np.float32(1.0))
            l23 = jnp.where(jnp.logical_or(between(32, 48), between(80, 96)), low[1], np.float32(1.0))
            safe = jnp.min(jnp.minimum(l01, l23)) >= np.float32(2.0 ** -60)

            @pl.when(jnp.logical_not(safe))
            def _redo():
                def one(c, carry):
                    stage_b2(qkv_r, att_w, c, stage_b1(qkv_r, c), True)
                    return carry
                jax.lax.fori_loop(0, NW, one, 0)

    r = pl.program_id(0)

    @pl.when(r == 0)
    def _first():
        prepare_weights()
        att_o[...] = jnp.ones(att_o.shape, F32)
        x0_o[pl.ds(slot(-1) * WS * 4, WS * 4)] = jnp.zeros((WS * 4, C, 128), F32)
        step(0, 0, 'A')

    @pl.when(r == 1)
    def _second():
        step(1, 1, 'AL')

    @pl.when(jnp.logical_and(r % 2 == 0, jnp.logical_and(r >= 2, r <= NW - 1)))
    def _even():
        step(r, 0, 'ABCL')

    @pl.when(jnp.logical_and(r % 2 == 1, jnp.logical_and(r >= 2, r <= NW)))
    def _odd():
        step(r, 1, 'ABCL')

    @pl.when(r == NW + 1)
    def _second_last():
        step(NW + 1, (NW + 1) % 2, 'BC')

    @pl.when(r == NW + 2)
    def _last():
        step(NW + 2, (NW + 2) % 2, 'C')


@jax.jit
def pallas_standalone__window_attn_davit__vision_kernel(
    x: jax.Array,
    dw_pe: jax.Array,
    w_qkv: jax.Array,
    w_o: jax.Array,
):
    xt = jnp.transpose(x.reshape(H, W, C), (0, 2, 1))
    dwt = jnp.transpose(dw_pe.reshape(9, C), (1, 0))
    full = lambda shape: pl.BlockSpec(shape, lambda r: (0,) * len(shape))
    out = pl.pallas_call(
        _kernel,
        grid=(NSTEP,),
        in_specs=[
            pl.BlockSpec((1, C, WP), lambda r: (jnp.maximum(jnp.minimum(r, NW - 1) * WS - 1, 0), 0, 0)),
            pl.BlockSpec((WS, C, WP), lambda r: (jnp.minimum(r, NW - 1), 0, 0)),
            pl.BlockSpec((1, C, WP), lambda r: (jnp.minimum(r * WS + WS, H - 1), 0, 0)),
            full((C, 9)),
            full((C, 3 * C)),
            full((C, C)),
        ],
        out_specs=pl.BlockSpec((WS, C, WP), lambda r: (jnp.maximum(r - 3, 0), 0, 0)),
        out_shape=jax.ShapeDtypeStruct((H, C, W), x.dtype),
        scratch_shapes=[
            pltpu.VMEM((C, 640), BF16),
            pltpu.VMEM((C, 256), BF16),
            pltpu.VMEM((9, C, 128), F32),
            pltpu.VMEM((2 * WS * 4, C, 128), F32),
            pltpu.VMEM((2 * WS * 4, C, 128), F32),
            pltpu.VMEM((5, WS * WP, 128), F32),
            pltpu.VMEM((5, WS * WP, 128), F32),
            pltpu.VMEM((2, WS * WP, 128), F32),
            pltpu.VMEM((2, WS * WP, 128), F32),
        ],
        compiler_params=pltpu.CompilerParams(
            dimension_semantics=("arbitrary",),
            vmem_limit_bytes=64 * 1024 * 1024,
        ),
    )(xt, xt, xt, dwt, w_qkv, w_o)
    return jnp.transpose(out, (0, 2, 1)).reshape(1, H, W, C)
```

```python
import functools
import os
import re
import numpy as np
import jax
import jax.numpy as jnp
import jax.experimental.pallas as pl
import jax.experimental.pallas.tpu as pltpu

WS = 7
NH = 4
C = 192
DH = C // NH
H = W = 511
WP = 512
NW = W // WS
NSTEP = NW + 3
EPS = 1e-05
NEG = -1e30
F32 = jnp.float32
BF16 = jnp.bfloat16
BLAG = int(os.environ.get('BLAG', '8'))
ORDER = os.environ.get('ORDER', 'B,L2,AL,C')


def _nt(a, b):
    return jax.lax.dot_general(a, b, (((1,), (1,)), ((), ())), preferred_element_type=F32)


def _nn(a, b):
    return jax.lax.dot_general(a, b, (((1,), (0,)), ((), ())), preferred_element_type=F32)


def _kernel(xt_ref, xm_ref, xb_ref, dw_hbm, wqkv_hbm, wo_hbm, o_ref,
            dw_ref, wqkv_ref, wo_ref, sems, wq_s, wo_s, dwb_s, x0_e, x0_o, qkv_e, qkv_o, att_e, att_o):
    lane16 = jax.lax.broadcasted_iota(jnp.int32, (16, 128), 1)
    l8 = jax.lax.broadcasted_iota(jnp.int32, (8, 128), 1)
    seg_a = l8 < 64
    key_ok = jnp.logical_and((l8 % 64) < 56, (l8 % 8) < 7)
    oka = jnp.logical_and(key_ok, seg_a)
    okb = jnp.logical_and(key_ok, jnp.logical_not(seg_a))
    z8 = jnp.zeros((8, 128), F32)

    def between(lo, hi):
        return jnp.logical_and(l8 >= lo, l8 < hi)

    def ones_at(lo, hi):
        return jnp.where(between(lo, hi), 1.0, 0.0).astype(F32)

    def slot(q):
        return ((q + 4) // 2) % 2

    def prepare_weights():
        copies = [pltpu.make_async_copy(src, dst, sems.at[j])
                  for j, (src, dst) in enumerate(((dw_hbm, dw_ref), (wqkv_hbm, wqkv_ref), (wo_hbm, wo_ref)))]
        for cp in copies:
            cp.start()
        for cp in copies:
            cp.wait()
        w = wqkv_ref[...].astype(F32)
        qs = w[:, 0:C] * np.float32(DH ** -0.5 * np.log2(np.e))
        q = [qs[:, h * DH:(h + 1) * DH] for h in range(NH)]
        k = [w[:, C + h * DH:C + (h + 1) * DH] for h in range(NH)]
        v = [w[:, 2 * C + h * DH:2 * C + (h + 1) * DH] for h in range(NH)]
        z32 = jnp.zeros((C, 32), F32)
        tiles = [
            [q[0], v[2][:, 32:48], v[3][:, 0:16], q[1]],
            [v[2][:, 0:32], q[2], q[3]],
            [k[0], z32, k[1]],
            [z32, k[2], k[3]],
            [v[0], v[1], v[3][:, 16:48]],
        ]
        for t in range(5):
            wq_s[:, t * 128:(t + 1) * 128] = jnp.concatenate(tiles[t], axis=1).astype(BF16)
        wo = wo_ref[...].astype(F32)
        zr = lambda n: jnp.zeros((n, C), F32)
        wo2 = jnp.concatenate([wo[0:96], zr(32), wo[96:128], zr(16), wo[128:160], zr(16), wo[160:192]], axis=0)
        wo_s[...] = wo2.T.astype(BF16)
        taps = [dw_ref[i].astype(F32) for i in range(3)]
        dw = jnp.concatenate([t[j:j + 1] for t in taps for j in range(3)] + [jnp.zeros((7, C), F32)], axis=0).T
        for j in range(9):
            col = dw[:, j:j + 1]
            if j == 4:
                col = col + 1.0
            dwb_s[j] = jnp.broadcast_to(col, (C, 128))

    def stage_a(r, x0_s, g, half):
        cs = pl.ds(g * 16, 16)
        co = pl.ds(g * 16 + half * 8, 8)
        base = slot(r) * (WS * 4)
        wts = [dwb_s[j, co, :] for j in range(9)]
        ra = min(r, NW - 1) if isinstance(r, int) else jnp.minimum(r, NW - 1)

        def load_row(i):
            if i == -1:
                v = jnp.where(ra > 0, xt_ref[0, cs, :].astype(F32), 0.0)
            elif i == WS:
                v = jnp.where(ra < NW - 1, xb_ref[0, cs, :].astype(F32), 0.0)
            else:
                v = xm_ref[i, cs, :].astype(F32)
            v = v[half * 8:(half + 1) * 8]
            parts = [v[:, t * 128:(t + 1) * 128] for t in range(4)]
            parts[3] = jnp.where(l8 < W - 3 * 128, parts[3], 0.0)
            return parts

        rows = {-1: load_row(-1), 0: load_row(0)}
        for i in range(WS):
            rows[i + 1] = load_row(i + 1)
            v0, v1, v2 = [], [], []
            for t in range(4):
                a, b, c = rows[i - 1][t], rows[i][t], rows[i + 1][t]
                v0.append(pltpu.roll(a * wts[0] + b * wts[3] + c * wts[6], 1, 1))
                v1.append(a * wts[1] + b * wts[4] + c * wts[7])
                v2.append(pltpu.roll(a * wts[2] + b * wts[5] + c * wts[8], 127, 1))
            for t in range(4):
                lf = jnp.where(l8 == 0, 0.0 if t == 0 else v0[t - 1], v0[t])
                rt = jnp.where(l8 == 127, 0.0 if t == 3 else v2[t + 1], v2[t])
                x0_s[base + (i * 4 + t), co, :] = v1[t] + lf + rt
            del rows[i - 1]

    def stage_l(r, x0_s, qkv_s, i, t):
        x0 = x0_s[slot(r - 1) * (WS * 4) + i * 4 + t]
        m = jnp.mean(x0, axis=0, keepdims=True)
        d = x0 - m
        var = jnp.mean(d * d, axis=0, keepdims=True)
        h = d * jax.lax.rsqrt(var + EPS)
        qkv = _nn(h.T.astype(BF16), wq_s[...])
        for j in range(5):
            qkv_s[j, pl.ds(i * WP + t * 128, 128), :] = qkv[:, j * 128:(j + 1) * 128]

    def ext(rows_a, rows_b):
        return jnp.concatenate(rows_a + [z8] + rows_b + [z8], axis=0).astype(BF16)

    def ld(qkv_s, t, c):
        return [qkv_s[t, pl.ds(i * WP + c * WS, 8), :] for i in range(WS)]

    def stage_b1(qkv_s, c):
        t2, t3 = ld(qkv_s, 2, c), ld(qkv_s, 3, c)
        k01 = ext([jnp.where(l8 < 48, x, 0.0) for x in t2], [jnp.where(l8 >= 80, x, 0.0) for x in t2])
        k23 = ext([jnp.where(between(32, 80), x, 0.0) for x in t3], [jnp.where(l8 >= 80, x, 0.0) for x in t3])
        q01 = jnp.concatenate(ld(qkv_s, 0, c), axis=0)
        q23 = jnp.concatenate(ld(qkv_s, 1, c), axis=0)
        return _nt(q01, k01), _nt(q23, k23)

    def stage_b2(qkv_s, att_s, c, ss, exact):
        outs = []
        for t, s in enumerate(ss):
            ps = []
            for i in range(WS):
                si = s[i * 8:(i + 1) * 8]
                if exact:
                    ma = jnp.max(jnp.where(oka, si, NEG), axis=1, keepdims=True)
                    mb = jnp.max(jnp.where(okb, si, NEG), axis=1, keepdims=True)
                    ps.append(jnp.exp2(jnp.where(key_ok, si - jnp.where(seg_a, ma, mb), NEG)))
                else:
                    sm = jnp.where(key_ok, si, NEG)
                    ps.append(jnp.exp2(sm - jnp.max(sm, axis=1, keepdims=True)))
            if t == 0:
                t4 = ld(qkv_s, 4, c)
                v = ext([jnp.where(l8 < 48, x, ones_at(96, 112)) for x in t4],
                        [jnp.where(between(48, 96), x, ones_at(112, 128)) for x in t4])
            else:
                t0, t1, t4 = ld(qkv_s, 0, c), ld(qkv_s, 1, c), ld(qkv_s, 4, c)
                v = ext([jnp.where(l8 < 32, b, jnp.where(between(48, 64), a, ones_at(32, 48))) for a, b in zip(t0, t1)],
                        [jnp.where(l8 >= 96, d, jnp.where(between(64, 80), a, ones_at(80, 96))) for a, d in zip(t0, t4)])
            o = _nn(jnp.concatenate(ps, axis=0), v)
            for i in range(WS):
                att_s[t, pl.ds(i * WP + c * WS, 8), :] = o[i * 8:(i + 1) * 8]
            outs.append(o)
        return outs

    def b_items(qkv_s, att_s, low):
        pend = {}

        def f1(c):
            pend[c] = stage_b1(qkv_s, c)

        def f2(c):
            for t, o in enumerate(stage_b2(qkv_s, att_s, c, pend.pop(c), False)):
                for i in range(WS):
                    oi = o[i * 8:(i + 1) * 8]
                    low[t] = oi if low[t] is None else jnp.minimum(low[t], oi)

        items = []
        for u in range(NW + BLAG):
            if u < NW:
                items.append(functools.partial(f1, u))
            if u >= BLAG:
                items.append(functools.partial(f2, u - BLAG))
        return items

    idx01 = jnp.where(l8 < 48, 96, 112)
    idx23 = jnp.where(l8 < 64, 32, 80)

    def stage_c(r, x0_s, att_s, i, t):
        parts = []
        for j, idx in enumerate((idx01, idx23)):
            a = att_s[j, pl.ds(i * WP + t * 128, 128), :]
            pieces = []
            for u in range(16):
                au = a[u * 8:(u + 1) * 8]
                pieces.append(au * pl.reciprocal(jnp.take_along_axis(au, idx, axis=1), approx=True))
            parts.append(jnp.concatenate(pieces, axis=0))
        o = jnp.concatenate(parts, axis=1).astype(BF16)
        y = _nt(wo_s[...], o)
        x0 = x0_s[slot(r - 3) * (WS * 4) + i * 4 + t]
        o_ref[i, :, t * 128:(t + 1) * 128] = (y + x0).astype(o_ref.dtype)

    def step(r, parity, stages, extra=()):
        x0_w, x0_r, qkv_w, qkv_r, att_w, att_r = (
            (x0_e, x0_o, qkv_o, qkv_e, att_e, att_o) if parity == 0 else (x0_o, x0_e, qkv_e, qkv_o, att_o, att_e))
        units = [(u % WS, u // WS) for u in range(4 * WS)]
        low = [None, None]
        items = {
            'A': [functools.partial(stage_a, r, x0_w, g, hf) for g in range(C // 16) for hf in range(2)],
            'L': [functools.partial(stage_l, r, x0_r, qkv_w, i, t) for i, t in units],
            'B': b_items(qkv_r, att_w, low),
            'C': [functools.partial(stage_c, r, x0_r, att_r, i, t) for i, t in units],
            'X': list(extra),
        }
        taken = {s: 0 for s in items}
        for group in ORDER.split(','):
            sel = []
            for s, cnt in re.findall(r'([ABCL])(\d*)', group):
                if s in stages:
                    e = len(items[s]) if not cnt else min(len(items[s]), taken[s] + int(cnt))
                    sel.append(items[s][taken[s]:e])
                    taken[s] = e
            if not sel:
                continue
            n_steps = max(len(q) for q in sel)
            pos = [0] * len(sel)
            for u in range(n_steps):
                for j, q in enumerate(sel):
                    e = -(-(u + 1) * len(q) // n_steps)
                    for f in q[pos[j]:e]:
                        f()
                    pos[j] = e
        for s in stages:
            assert taken[s] == len(items[s])
        if 'B' in stages:
            l01 = jnp.where(l8 >= 96, low[0], np.float32(1.0))
            l23 = jnp.where(jnp.logical_or(between(32, 48), between(80, 96)), low[1], np.float32(1.0))
            safe = jnp.min(jnp.minimum(l01, l23)) >= np.float32(2.0 ** -60)

            @pl.when(jnp.logical_not(safe))
            def _redo():
                def one(c, carry):
                    stage_b2(qkv_r, att_w, c, stage_b1(qkv_r, c), True)
                    return carry
                jax.lax.fori_loop(0, NW, one, 0)

    r = pl.program_id(0)

    @pl.when(r == 0)
    def _first():
        prepare_weights()
        att_o[...] = jnp.ones(att_o.shape, F32)
        x0_o[pl.ds(slot(-1) * WS * 4, WS * 4)] = jnp.zeros((WS * 4, C, 128), F32)
        step(0, 0, 'A')

    @pl.when(r == 1)
    def _second():
        step(1, 1, 'AL')

    @pl.when(jnp.logical_and(r % 2 == 0, jnp.logical_and(r >= 2, r <= NW - 1)))
    def _even():
        step(r, 0, 'ABCL')

    @pl.when(jnp.logical_and(r % 2 == 1, jnp.logical_and(r >= 2, r <= NW)))
    def _odd():
        step(r, 1, 'ABCL')

    @pl.when(r == NW + 1)
    def _second_last():
        step(NW + 1, (NW + 1) % 2, 'BC')

    @pl.when(r == NW + 2)
    def _last():
        step(NW + 2, (NW + 2) % 2, 'C')


@jax.jit
def pallas_standalone__window_attn_davit__vision_kernel(
    x: jax.Array,
    dw_pe: jax.Array,
    w_qkv: jax.Array,
    w_o: jax.Array,
):
    xt = jnp.transpose(x.reshape(H, W, C), (0, 2, 1))
    full = lambda shape: pl.BlockSpec(shape, lambda r: (0,) * len(shape))
    out = pl.pallas_call(
        _kernel,
        grid=(NSTEP,),
        in_specs=[
            pl.BlockSpec((1, C, WP), lambda r: (jnp.maximum(jnp.minimum(r, NW - 1) * WS - 1, 0), 0, 0)),
            pl.BlockSpec((WS, C, WP), lambda r: (jnp.minimum(r, NW - 1), 0, 0)),
            pl.BlockSpec((1, C, WP), lambda r: (jnp.minimum(r * WS + WS, H - 1), 0, 0)),
            pl.BlockSpec(memory_space=pl.ANY),
            pl.BlockSpec(memory_space=pl.ANY),
            pl.BlockSpec(memory_space=pl.ANY),
        ],
        out_specs=pl.BlockSpec((WS, C, WP), lambda r: (jnp.maximum(r - 3, 0), 0, 0)),
        out_shape=jax.ShapeDtypeStruct((H, C, W), x.dtype),
        scratch_shapes=[
            pltpu.VMEM((3, 3, C), BF16),
            pltpu.VMEM((C, 3 * C), BF16),
            pltpu.VMEM((C, C), BF16),
            pltpu.SemaphoreType.DMA((3,)),
            pltpu.VMEM((C, 640), BF16),
            pltpu.VMEM((C, 256), BF16),
            pltpu.VMEM((9, C, 128), F32),
            pltpu.VMEM((2 * WS * 4, C, 128), F32),
            pltpu.VMEM((2 * WS * 4, C, 128), F32),
            pltpu.VMEM((5, WS * WP, 128), F32),
            pltpu.VMEM((5, WS * WP, 128), F32),
            pltpu.VMEM((2, WS * WP, 128), F32),
            pltpu.VMEM((2, WS * WP, 128), F32),
        ],
        compiler_params=pltpu.CompilerParams(
            dimension_semantics=("arbitrary",),
            vmem_limit_bytes=64 * 1024 * 1024,
        ),
    )(xt, xt, xt, dw_pe, w_qkv, w_o)
    return jnp.transpose(out, (0, 2, 1)).reshape(1, H, W, C)
```

```python
import functools
import numpy as np
import jax
import jax.numpy as jnp
import jax.experimental.pallas as pl
import jax.experimental.pallas.tpu as pltpu

WS = 7
NH = 4
C = 192
DH = C // NH
H = W = 511
WP = 512
NW = W // WS
NSTEP = NW + 3
EPS = 1e-05
NEG = float('-inf')
F32 = jnp.float32
BF16 = jnp.bfloat16
BLAG = 8
ORDER = ((('B', None),), (('L', 2),), (('A', None), ('L', None)), (('C', None),))


def _nt(a, b):
    return jax.lax.dot_general(a, b, (((1,), (1,)), ((), ())), preferred_element_type=F32)


def _nn(a, b):
    return jax.lax.dot_general(a, b, (((1,), (0,)), ((), ())), preferred_element_type=F32)


def _kernel(xt_ref, xm_ref, xb_ref, dw_hbm, wqkv_hbm, wo_hbm, o_ref,
            dw_ref, wqkv_ref, wo_ref, sems, wq_s, wo_s, dwb_s, x0_e, x0_o, qkv_e, qkv_o, att_e, att_o):
    l8 = jax.lax.broadcasted_iota(jnp.int32, (8, 128), 1)
    seg_a = l8 < 64
    key_ok = jnp.logical_and((l8 % 64) < 56, (l8 % 8) < 7)
    oka = jnp.logical_and(key_ok, seg_a)
    okb = jnp.logical_and(key_ok, jnp.logical_not(seg_a))
    z8 = jnp.zeros((8, 128), F32)

    def between(lo, hi):
        return jnp.logical_and(l8 >= lo, l8 < hi)

    def ones_at(lo, hi):
        return jnp.where(between(lo, hi), 1.0, 0.0).astype(F32)

    def slot(q):
        return ((q + 4) // 2) % 2

    def prepare_weights():
        copies = [pltpu.make_async_copy(src, dst, sems.at[j])
                  for j, (src, dst) in enumerate(((dw_hbm, dw_ref), (wqkv_hbm, wqkv_ref), (wo_hbm, wo_ref)))]
        for cp in copies:
            cp.start()
        for cp in copies:
            cp.wait()
        w = wqkv_ref[...].astype(F32)
        qs = w[:, 0:C] * np.float32(DH ** -0.5 * np.log2(np.e))
        q = [qs[:, h * DH:(h + 1) * DH] for h in range(NH)]
        k = [w[:, C + h * DH:C + (h + 1) * DH] for h in range(NH)]
        v = [w[:, 2 * C + h * DH:2 * C + (h + 1) * DH] for h in range(NH)]
        z32 = jnp.zeros((C, 32), F32)
        tiles = [
            [q[0], v[2][:, 32:48], v[3][:, 0:16], q[1]],
            [v[2][:, 0:32], q[2], q[3]],
            [k[0], z32, k[1]],
            [z32, k[2], k[3]],
            [v[0], v[1], v[3][:, 16:48]],
        ]
        for t in range(5):
            wq_s[:, t * 128:(t + 1) * 128] = jnp.concatenate(tiles[t], axis=1).astype(BF16)
        wo = wo_ref[...].astype(F32)
        zr = lambda n: jnp.zeros((n, C), F32)
        wo2 = jnp.concatenate([wo[0:96], zr(32), wo[96:128], zr(16), wo[128:160], zr(16), wo[160:192]], axis=0)
        wo_s[...] = wo2.T.astype(BF16)
        taps = [dw_ref[i].astype(F32) for i in range(3)]
        dw = jnp.concatenate([t[j:j + 1] for t in taps for j in range(3)] + [jnp.zeros((7, C), F32)], axis=0).T
        for j in range(9):
            col = dw[:, j:j + 1]
            if j == 4:
                col = col + 1.0
            dwb_s[j] = jnp.broadcast_to(col, (C, 128))

    def stage_a(r, x0_s, g, half):
        cs = pl.ds(g * 16, 16)
        co = pl.ds(g * 16 + half * 8, 8)
        base = slot(r) * (WS * 4)
        wts = [dwb_s[j, co, :] for j in range(9)]
        ra = min(r, NW - 1) if isinstance(r, int) else jnp.minimum(r, NW - 1)

        def load_row(i):
            if i == -1:
                v = jnp.where(ra > 0, xt_ref[0, cs, :].astype(F32), 0.0)
            elif i == WS:
                v = jnp.where(ra < NW - 1, xb_ref[0, cs, :].astype(F32), 0.0)
            else:
                v = xm_ref[i, cs, :].astype(F32)
            v = v[half * 8:(half + 1) * 8]
            parts = [v[:, t * 128:(t + 1) * 128] for t in range(4)]
            parts[3] = jnp.where(l8 < W - 3 * 128, parts[3], 0.0)
            return parts

        rows = {-1: load_row(-1), 0: load_row(0)}
        for i in range(WS):
            rows[i + 1] = load_row(i + 1)
            v0, v1, v2 = [], [], []
            for t in range(4):
                a, b, c = rows[i - 1][t], rows[i][t], rows[i + 1][t]
                v0.append(pltpu.roll(a * wts[0] + b * wts[3] + c * wts[6], 1, 1))
                v1.append(a * wts[1] + b * wts[4] + c * wts[7])
                v2.append(pltpu.roll(a * wts[2] + b * wts[5] + c * wts[8], 127, 1))
            for t in range(4):
                lf = jnp.where(l8 == 0, 0.0 if t == 0 else v0[t - 1], v0[t])
                rt = jnp.where(l8 == 127, 0.0 if t == 3 else v2[t + 1], v2[t])
                x0_s[base + (i * 4 + t), co, :] = v1[t] + lf + rt
            del rows[i - 1]

    def stage_l(r, x0_s, qkv_s, i, t):
        x0 = x0_s[slot(r - 1) * (WS * 4) + i * 4 + t]
        m = jnp.mean(x0, axis=0, keepdims=True)
        d = x0 - m
        var = jnp.mean(d * d, axis=0, keepdims=True)
        h = d * jax.lax.rsqrt(var + EPS)
        qkv = _nn(h.T.astype(BF16), wq_s[...])
        for j in range(5):
            qkv_s[j, pl.ds(i * WP + t * 128, 128), :] = qkv[:, j * 128:(j + 1) * 128]

    def ext(rows_a, rows_b):
        return jnp.concatenate(rows_a + [z8] + rows_b + [z8], axis=0).astype(BF16)

    def ld(qkv_s, t, c):
        return [qkv_s[t, pl.ds(i * WP + c * WS, 8), :] for i in range(WS)]

    def stage_b1(qkv_s, c):
        t2, t3 = ld(qkv_s, 2, c), ld(qkv_s, 3, c)
        k01 = ext([jnp.where(l8 < 48, x, 0.0) for x in t2], [jnp.where(l8 >= 80, x, 0.0) for x in t2])
        k23 = ext([jnp.where(between(32, 80), x, 0.0) for x in t3], [jnp.where(l8 >= 80, x, 0.0) for x in t3])
        q01 = jnp.concatenate(ld(qkv_s, 0, c), axis=0)
        q23 = jnp.concatenate(ld(qkv_s, 1, c), axis=0)
        return _nt(q01, k01), _nt(q23, k23)

    def stage_b2(qkv_s, att_s, c, ss, exact):
        outs = []
        for t, s in enumerate(ss):
            ps = []
            for i in range(WS):
                si = s[i * 8:(i + 1) * 8]
                if exact:
                    ma = jnp.max(jnp.where(oka, si, NEG), axis=1, keepdims=True)
                    mb = jnp.max(jnp.where(okb, si, NEG), axis=1, keepdims=True)
                    ps.append(jnp.exp2(jnp.where(key_ok, si - jnp.where(seg_a, ma, mb), NEG)))
                else:
                    sm = jnp.where(key_ok, si, NEG)
                    ps.append(jnp.exp2(sm - jnp.max(sm, axis=1, keepdims=True)))
            if t == 0:
                t4 = ld(qkv_s, 4, c)
                v = ext([jnp.where(l8 < 48, x, ones_at(96, 112)) for x in t4],
                        [jnp.where(between(48, 96), x, ones_at(112, 128)) for x in t4])
            else:
                t0, t1, t4 = ld(qkv_s, 0, c), ld(qkv_s, 1, c), ld(qkv_s, 4, c)
                v = ext([jnp.where(l8 < 32, b, jnp.where(between(48, 64), a, ones_at(32, 48))) for a, b in zip(t0, t1)],
                        [jnp.where(l8 >= 96, d, jnp.where(between(64, 80), a, ones_at(80, 96))) for a, d in zip(t0, t4)])
            o = _nn(jnp.concatenate(ps, axis=0), v)
            for i in range(WS):
                att_s[t, pl.ds(i * WP + c * WS, 8), :] = o[i * 8:(i + 1) * 8]
            outs.append(o)
        return outs

    def b_items(qkv_s, att_s, low):
        pend = {}

        def f1(c):
            pend[c] = stage_b1(qkv_s, c)

        def f2(c):
            for t, o in enumerate(stage_b2(qkv_s, att_s, c, pend.pop(c), False)):
                for i in range(WS):
                    oi = o[i * 8:(i + 1) * 8]
                    low[t] = oi if low[t] is None else jnp.minimum(low[t], oi)

        items = []
        for u in range(NW + BLAG):
            if u < NW:
                items.append(functools.partial(f1, u))
            if u >= BLAG:
                items.append(functools.partial(f2, u - BLAG))
        return items

    idx01 = jnp.where(l8 < 48, 96, 112)
    idx23 = jnp.where(l8 < 64, 32, 80)

    def stage_c(r, x0_s, att_s, i, t):
        parts = []
        for j, idx in enumerate((idx01, idx23)):
            a = att_s[j, pl.ds(i * WP + t * 128, 128), :]
            pieces = []
            for u in range(16):
                au = a[u * 8:(u + 1) * 8]
                pieces.append(au * pl.reciprocal(jnp.take_along_axis(au, idx, axis=1), approx=True))
            parts.append(jnp.concatenate(pieces, axis=0))
        o = jnp.concatenate(parts, axis=1).astype(BF16)
        y = _nt(wo_s[...], o)
        x0 = x0_s[slot(r - 3) * (WS * 4) + i * 4 + t]
        o_ref[i, :, t * 128:(t + 1) * 128] = (y + x0).astype(o_ref.dtype)

    def step(r, parity, stages):
        x0_w, x0_r, qkv_w, qkv_r, att_w, att_r = (
            (x0_e, x0_o, qkv_o, qkv_e, att_e, att_o) if parity == 0 else (x0_o, x0_e, qkv_e, qkv_o, att_o, att_e))
        units = [(u % WS, u // WS) for u in range(4 * WS)]
        low = [None, None]
        items = {
            'A': [functools.partial(stage_a, r, x0_w, g, hf) for g in range(C // 16) for hf in range(2)],
            'L': [functools.partial(stage_l, r, x0_r, qkv_w, i, t) for i, t in units],
            'B': b_items(qkv_r, att_w, low),
            'C': [functools.partial(stage_c, r, x0_r, att_r, i, t) for i, t in units],
        }
        taken = {s: 0 for s in items}
        for group in ORDER:
            sel = []
            for s, cnt in group:
                if s in stages:
                    e = len(items[s]) if cnt is None else min(len(items[s]), taken[s] + cnt)
                    sel.append(items[s][taken[s]:e])
                    taken[s] = e
            if not sel:
                continue
            n_steps = max(len(q) for q in sel)
            pos = [0] * len(sel)
            for u in range(n_steps):
                for j, q in enumerate(sel):
                    e = -(-(u + 1) * len(q) // n_steps)
                    for f in q[pos[j]:e]:
                        f()
                    pos[j] = e
        for s in stages:
            assert taken[s] == len(items[s])
        if 'B' in stages:
            l01 = jnp.where(l8 >= 96, low[0], np.float32(1.0))
            l23 = jnp.where(jnp.logical_or(between(32, 48), between(80, 96)), low[1], np.float32(1.0))
            safe = jnp.min(jnp.minimum(l01, l23)) >= np.float32(2.0 ** -30)

            @pl.when(jnp.logical_not(safe))
            def _redo():
                def one(c, carry):
                    stage_b2(qkv_r, att_w, c, stage_b1(qkv_r, c), True)
                    return carry
                jax.lax.fori_loop(0, NW, one, 0)

    r = pl.program_id(0)

    @pl.when(r == 0)
    def _first():
        prepare_weights()
        att_o[...] = jnp.ones(att_o.shape, F32)
        x0_o[pl.ds(slot(-1) * WS * 4, WS * 4)] = jnp.zeros((WS * 4, C, 128), F32)
        step(0, 0, 'A')

    @pl.when(r == 1)
    def _second():
        step(1, 1, 'AL')

    @pl.when(jnp.logical_and(r % 2 == 0, jnp.logical_and(r >= 2, r <= NW - 1)))
    def _even():
        step(r, 0, 'ABCL')

    @pl.when(jnp.logical_and(r % 2 == 1, jnp.logical_and(r >= 2, r <= NW)))
    def _odd():
        step(r, 1, 'ABCL')

    @pl.when(r == NW + 1)
    def _second_last():
        step(NW + 1, (NW + 1) % 2, 'BC')

    @pl.when(r == NW + 2)
    def _last():
        step(NW + 2, (NW + 2) % 2, 'C')


@jax.jit
def pallas_standalone__window_attn_davit__vision_kernel(
    x: jax.Array,
    dw_pe: jax.Array,
    w_qkv: jax.Array,
    w_o: jax.Array,
):
    xt = jnp.transpose(x.reshape(H, W, C), (0, 2, 1))
    out = pl.pallas_call(
        _kernel,
        grid=(NSTEP,),
        in_specs=[
            pl.BlockSpec((1, C, WP), lambda r: (jnp.maximum(jnp.minimum(r, NW - 1) * WS - 1, 0), 0, 0)),
            pl.BlockSpec((WS, C, WP), lambda r: (jnp.minimum(r, NW - 1), 0, 0)),
            pl.BlockSpec((1, C, WP), lambda r: (jnp.minimum(r * WS + WS, H - 1), 0, 0)),
            pl.BlockSpec(memory_space=pl.ANY),
            pl.BlockSpec(memory_space=pl.ANY),
            pl.BlockSpec(memory_space=pl.ANY),
        ],
        out_specs=pl.BlockSpec((WS, C, WP), lambda r: (jnp.maximum(r - 3, 0), 0, 0)),
        out_shape=jax.ShapeDtypeStruct((H, C, W), x.dtype),
        scratch_shapes=[
            pltpu.VMEM((3, 3, C), BF16),
            pltpu.VMEM((C, 3 * C), BF16),
            pltpu.VMEM((C, C), BF16),
            pltpu.SemaphoreType.DMA((3,)),
            pltpu.VMEM((C, 640), BF16),
            pltpu.VMEM((C, 256), BF16),
            pltpu.VMEM((9, C, 128), F32),
            pltpu.VMEM((2 * WS * 4, C, 128), F32),
            pltpu.VMEM((2 * WS * 4, C, 128), F32),
            pltpu.VMEM((5, WS * WP, 128), F32),
            pltpu.VMEM((5, WS * WP, 128), F32),
            pltpu.VMEM((2, WS * WP, 128), F32),
            pltpu.VMEM((2, WS * WP, 128), F32),
        ],
        compiler_params=pltpu.CompilerParams(
            dimension_semantics=("arbitrary",),
            vmem_limit_bytes=64 * 1024 * 1024,
        ),
    )(xt, xt, xt, dw_pe, w_qkv, w_o)
    return jnp.transpose(out, (0, 2, 1)).reshape(1, H, W, C)
```
